```python
import os as _os
_os.environ.setdefault("JAX_PLATFORMS", "cpu")
import jax
import jax.numpy as jnp

def _softmax(x, axis=-1):
    return jax.nn.softmax(x, axis=axis)
def _gelu(x):
    return jax.nn.gelu(x, approximate=True)
def _silu(x):
    return jax.nn.silu(x)
def _sigmoid(x):
    return jax.nn.sigmoid(x)
def _layernorm(x, axis=-1, eps=1e-5):
    m = jnp.mean(x, axis=axis, keepdims=True)
    v = jnp.var(x, axis=axis, keepdims=True)
    return (x - m) / jnp.sqrt(v + eps)
def _scatter_add(tgt, idx, src, axis=0):
    return tgt.at[idx].add(src)
def _segment_sum(src, seg, n):
    return jax.ops.segment_sum(src, seg, n)
class _Rng:
    def __init__(self, key):
        self._k = key
    def _next(self):
        self._k, sub = jax.random.split(self._k)
        return sub
    def normal(self, shape):
        return jax.random.normal(self._next(), shape, dtype=jnp.bfloat16)
    def randint(self, lo, hi, shape):
        return jax.random.randint(self._next(), shape, lo, hi, dtype=jnp.int32)
    def uniform(self, shape, lo=0.0, hi=1.0):
        return jax.random.uniform(self._next(), shape, jnp.bfloat16, lo, hi)
    def permutation(self, n):
        return jax.random.permutation(self._next(), n)


kernel_name = 'parallel_sum__ssm_conv_s5__geglu_ffn__prompt'

def setup_inputs():
    _rng = _Rng(jax.random.key(int.from_bytes(__import__("os").urandom(4), "little")))
    _w = (lambda a: (lambda t: t.astype(jnp.bfloat16) if jnp.issubdtype(t.dtype, jnp.floating) else t)(jnp.asarray(a)))
    def _A_setup():
        B, S, D = 1, 2048, 512
        P = D
        Lambda_re = -0.5 * jnp.exp((lambda *s: _rng.normal(s) * 0.8)(P))
        Lambda_im = (lambda *s: _rng.normal(s) * 0.8)(P) * 1.0
        B_re = (lambda *s: _rng.normal(s) * 0.8)(P, D) * (D ** -0.5)
        B_im = (lambda *s: _rng.normal(s) * 0.8)(P, D) * (D ** -0.5)
        C_re = (lambda *s: _rng.normal(s) * 0.8)(D, P) * (P ** -0.5)
        C_im = (lambda *s: _rng.normal(s) * 0.8)(D, P) * (P ** -0.5)
        log_dt = (lambda *s: _rng.normal(s) * 0.8)(P) * 0.3 - 2.0
        Dskip = (lambda *s: _rng.normal(s) * 0.8)(D)
        return {
            "x": _w((lambda *s: _rng.normal(s) * 0.05)(B, S, D)),
            "Lambda_re": _w(Lambda_re),
            "Lambda_im": _w(Lambda_im),
            "B_re": _w(B_re),
            "B_im": _w(B_im),
            "C_re": _w(C_re),
            "C_im": _w(C_im),
            "log_dt": _w(log_dt),
            "Dskip": _w(Dskip),
        }
    _A_in = _A_setup()

    def _B_setup():
        B, S, D, F = 1, 2048, 512, 1376
        return {
            "x": _w((lambda *s: _rng.normal(s) * 0.05)(B, S, D)),
            "w_gate": _w((lambda *s: _rng.normal(s) * 0.05)(D, F)),
            "w_up": _w((lambda *s: _rng.normal(s) * 0.05)(D, F)),
            "w_down": _w((lambda *s: _rng.normal(s) * 0.05)(F, D)),
        }
    _B_in = _B_setup()

    return {
        "A_x": _A_in["x"],
        "A_Lambda_re": _A_in["Lambda_re"],
        "A_Lambda_im": _A_in["Lambda_im"],
        "A_B_re": _A_in["B_re"],
        "A_B_im": _A_in["B_im"],
        "A_C_re": _A_in["C_re"],
        "A_C_im": _A_in["C_im"],
        "A_log_dt": _A_in["log_dt"],
        "A_Dskip": _A_in["Dskip"],
        "B_x": _B_in["x"],
        "B_w_gate": _B_in["w_gate"],
        "B_w_up": _B_in["w_up"],
        "B_w_down": _B_in["w_down"],
    }

def reference(A_x, A_Lambda_re, A_Lambda_im, A_B_re, A_B_im, A_C_re, A_C_im, A_log_dt, A_Dskip, B_x, B_w_gate, B_w_up, B_w_down):
    def _A_ref(x, Lambda_re, Lambda_im, B_re, B_im, C_re, C_im, log_dt, Dskip):
        Bsz, L, H = x.shape
        Lam = Lambda_re + 1j * Lambda_im
        Bmat = B_re + 1j * B_im
        Cmat = C_re + 1j * C_im
        dt = jnp.exp(log_dt)
        Lam_bar = jnp.exp(dt * Lam)
        B_bar = ((Lam_bar - 1.0) / Lam)[:, None] * Bmat
        Bu = jnp.einsum("bld,pd->blp", x + 0j, B_bar)
        h = jnp.zeros_like(Bu[:, 0, :])
        hs = []
        for t in range(L):
            h = Lam_bar[None, :] * h + Bu[:, t, :]
            hs.append(h)
        hseq = jnp.stack(hs, 1)
        y = 2.0 * jnp.einsum("blp,dp->bld", hseq, Cmat).real + x * Dskip[None, None, :]
        return y

    def _B_ref(x, w_gate, w_up, w_down):
        return (_gelu(x @ w_gate) * (x @ w_up)) @ w_down

    x = A_x
    xn = _layernorm(x, axis=-1)
    return x + _A_ref(xn, A_Lambda_re, A_Lambda_im, A_B_re, A_B_im, A_C_re, A_C_im, A_log_dt, A_Dskip) + _B_ref(xn, B_w_gate, B_w_up, B_w_down)
```

```python
import jax
import jax.numpy as jnp
from jax import lax
import jax.experimental.pallas as pl
import jax.experimental.pallas.tpu as pltpu

LS = (62, 66)
NIT = 2
PCOL = dict(bim=1, wg=2, wu=5, wd=5, x=9)
FL = {"XLA_TPU_RESCHEDULE_DMA_DONES": True}
NSER = (1, 12)
SDEL = (None, 3)
XBA = 0
NT = (((1,), (1,)), ((), ()))
f32 = jnp.float32
bf16 = jnp.bfloat16
u32 = jnp.uint32
PADR = 16
TA = 8 * max(LS)


def _gelu(x):
    c = 0.7978845608028654
    return 0.5 * x * (1.0 + jnp.tanh(c * (x + 0.044715 * (x * x * x))))


def _cmul(ar, ai, br, bi):
    return ar * br - ai * bi, ar * bi + ai * br


def _row(v):
    return jnp.concatenate([v[j:j + 1, :] for j in range(v.shape[0])], axis=1)


def _zero_of(v):
    z = lax.shift_right_logical(lax.clz(pltpu.bitcast(v[0:8, 0:128], u32)), jnp.uint32(6))
    return z[0:1, 0:1]


def _after(v, z):
    return pltpu.bitcast(pltpu.bitcast(v, u32) | z, f32)


def kernel(x_hbm, lre_hbm, lim_hbm, bre_hbm, bim_hbm, cre_hbm, cim_hbm, ldt_hbm, dsk_hbm,
           wg_hbm, wu_hbm, wd_hbm, o_hbm,
           x_v, vec_v, bre_v, bim_f, cre_v, cim_v, wg_f, wu_f, wd_f, o_v, tab_v, xb_s, sems):
    S, D = x_hbm.shape
    P = D
    F = wg_hbm.shape[0]
    NC = D // 128
    TS = [8 * l for l in LS]
    TI = sum(TS)
    assert TI * NIT == S
    OFF = [0, TS[0]]

    cnt = [0]

    def nsem(n=1):
        cnt[0] += n
        return cnt[0] - n

    def cp(src, dst, k):
        return pltpu.make_async_copy(src, dst, sems.at[k])

    bim_v = bim_f.at[pl.ds(0, P)]
    wg_v, wu_v, wd_v = wg_f.at[pl.ds(0, F)], wu_f.at[pl.ds(0, F)], wd_f.at[pl.ds(0, F)]
    DUM = F + PADR
    STG = DUM + NIT * PADR
    xa_v = wu_f.at[pl.ds(STG, TA)]
    xb_v = wd_f.at[pl.ds(STG, TA)] if XBA == 0 else xb_s

    XS = {t: nsem(NC) for t in range(2 * NIT)}
    OS0 = nsem(2 * NIT * NC)
    AS0 = nsem(NIT)

    def xcps(t):
        r, n = (t // 2) * TI + OFF[t % 2], TS[t % 2]
        return [cp(x_hbm.at[pl.ds(r, n), pl.ds(c * 128, 128)], x_v.at[c, pl.ds(r, n)], XS[t] + c) for c in range(NC)]

    def ocp(it, j, c):
        r = it * TI + OFF[j]
        if not isinstance(it, int):
            r = pl.multiple_of(r, 16)
        return cp(o_v.at[c, pl.ds(r, TS[j])], o_hbm.at[pl.ds(r, TS[j]), pl.ds(c * 128, 128)],
                  OS0 + (it * 2 + j) * NC + c)

    def acp(it):
        r = DUM + it * PADR
        if not isinstance(it, int):
            r = pl.multiple_of(r, PADR)
        return cp(wu_hbm.at[pl.ds(0, PADR)], wu_f.at[pl.ds(r, PADR)], AS0 + it)

    G = dict(
        vec=[cp(lre_hbm, vec_v.at[0], nsem()), cp(lim_hbm, vec_v.at[1], nsem()),
             cp(ldt_hbm, vec_v.at[2], nsem()), cp(dsk_hbm, vec_v.at[3], nsem())],
        x0=xcps(0),
        bre=[cp(bre_hbm, bre_v, nsem())], bim=[cp(bim_hbm, bim_v, nsem())],
        wg=[cp(wg_hbm, wg_v, nsem())], wu=[cp(wu_hbm, wu_v, nsem())],
        wd=[cp(wd_hbm, wd_v, nsem()), cp(cre_hbm, cre_v, nsem()), cp(cim_hbm, cim_v, nsem())],
        x=[c for t in range(1, 2 * NIT) for c in xcps(t)],
    )
    for n in ("vec", "x0", "bre", "bim", "wg", "wu", "wd", "x"):
        for c in G[n]:
            c.start()
    for it in range(NIT):
        acp(it).start()

    def wait(n):
        for c in G[n]:
            c.wait()

    def pin_wait(it, n, val, j):
        v = val[val.shape[0] - 16:, j * 128:(j + 1) * 128].astype(bf16)
        spare = dict(bim=bim_f.at[pl.ds(P, PADR), pl.ds(0, 128)], wg=wg_f.at[pl.ds(F, PADR), pl.ds(0, 128)],
                     wu=wu_f.at[pl.ds(F, PADR), pl.ds(0, 128)], wd=wd_f.at[pl.ds(F, PADR), pl.ds(0, 128)],
                     x=x_v.at[0, pl.ds(S, PADR)])[n]
        spare[...] = v

        @pl.when(it == 0)
        def _():
            wait(n)

    wait("vec")
    wait("x0")

    lre = vec_v[0].astype(f32)
    lim = vec_v[1].astype(f32)
    dt = jnp.exp(vec_v[2].astype(f32)).astype(bf16).astype(f32)
    wr = dt * lre
    wi = dt * lim
    mag = jnp.exp(wr)
    a_r = mag * jnp.cos(wi)
    a_i = mag * jnp.sin(wi)
    den = lre * lre + lim * lim
    nr = a_r - 1.0
    cf_r = 2.0 * ((nr * lre + a_i * lim) / den)
    cf_i = 2.0 * ((a_i * lre - nr * lim) / den)
    bc = lambda v: jnp.broadcast_to(_row(v), (8, P))
    row = lax.broadcasted_iota(jnp.int32, (8, P), 0)
    tab_v[0], tab_v[1] = bc(a_r), bc(a_i)
    tab_v[2], tab_v[3], tab_v[4] = bc(cf_r), bc(cf_i), bc(-cf_r)
    tab_v[5] = bc(vec_v[3].astype(f32))
    for j, Ls in enumerate(LS):
        magL = jnp.exp(Ls * wr)
        Ar, Ai = bc(magL * jnp.cos(Ls * wi)), bc(magL * jnp.sin(Ls * wi))
        A2 = _cmul(Ar, Ai, Ar, Ai)
        A4 = _cmul(*A2, *A2)
        b = 6 + 8 * j
        tab_v[b], tab_v[b + 1] = Ar, Ai
        for q, (s, (mr, mi)) in enumerate(((1, (Ar, Ai)), (2, A2), (4, A4))):
            tab_v[b + 2 + 2 * q] = jnp.where(row >= s, mr, 0.0)
            tab_v[b + 3 + 2 * q] = jnp.where(row >= s, mi, 0.0)

    xw = [x_v.at[c].bitcast(u32) for c in range(NC)]

    def xload(base2, j):
        Ls = LS[j]
        if not isinstance(base2, int):
            base2 = pl.multiple_of(base2, 8)
        xt = [xw[c].at[pl.ds(base2, 4 * Ls)] for c in range(NC)]
        parts = []
        for k in range(Ls // 2):
            w = jnp.concatenate([xt[c][pl.ds(k, 8, stride=Ls // 2), :] for c in range(NC)], axis=1)
            parts.append(pltpu.bitcast(w << 16, f32))
            parts.append(pltpu.bitcast(w & jnp.uint32(0xFFFF0000), f32))
        return jnp.concatenate(parts, axis=0)

    def ln(base2, j, nser=1):
        x = xload(base2, j)
        nb = x.shape[0] // 16
        edges = [16 * ((nb * q) // nser) for q in range(nser + 1)]
        outs, z = [], None
        for q in range(nser):
            xq = x[edges[q]:edges[q + 1]]
            m = jnp.mean(xq, axis=-1, keepdims=True)
            if z is not None:
                m = _after(m, z)
            xc = xq - m
            v = jnp.mean(xc * xc, axis=-1, keepdims=True)
            xn = xc * lax.rsqrt(v + 1e-5)
            z = _zero_of(xn)
            outs.append(xn.astype(bf16))
        return jnp.concatenate(outs, axis=0) if nser > 1 else outs[0]

    def scan(j, ur, ui, carry, z=None):
        Ls = LS[j]
        b = 6 + 8 * j
        us = [(ur[8 * k:8 * k + 8], ui[8 * k:8 * k + 8]) for k in range(Ls)]
        ar, ai = tab_v[0], tab_v[1]
        er, ei = us[0]
        if z is not None:
            er, ei = _after(er, z), _after(ei, z)
        for k in range(1, Ls):
            tr, ti = _cmul(ar, ai, er, ei)
            er, ei = tr + us[k][0], ti + us[k][1]
        zr = jnp.where(row == 0, carry[0], pltpu.roll(er, 1, 0))
        zi = jnp.where(row == 0, carry[1], pltpu.roll(ei, 1, 0))
        for t, sh in enumerate((1, 2, 4)):
            tr, ti = _cmul(tab_v[b + 2 + 2 * t], tab_v[b + 3 + 2 * t], pltpu.roll(zr, sh, 0), pltpu.roll(zi, sh, 0))
            zr, zi = zr + tr, zi + ti
        tr, ti = _cmul(tab_v[b], tab_v[b + 1], zr, zi)
        carry = (pltpu.roll(tr + er, 1, 0), pltpu.roll(ti + ei, 1, 0))
        hr, hi = zr, zi
        hrs, his = [], []
        cr, ci, ncr = tab_v[2], tab_v[3], tab_v[4]
        for k in range(Ls):
            tr, ti = _cmul(ar, ai, hr, hi)
            hr, hi = tr + us[k][0], ti + us[k][1]
            hrs.append(cr * hr - ci * hi)
            his.append(ncr * hi - ci * hr)
        return jnp.concatenate(hrs, axis=0).astype(bf16), jnp.concatenate(his, axis=0).astype(bf16), carry

    def tile(it, j, carry, first, ln_early, ln_late):
        T = TS[j]
        Ls = LS[j]
        base2 = it * (TI // 2) + OFF[j] // 2
        xs_v = (xa_v, xb_v)[j].at[pl.ds(0, T)]
        ur = lax.dot_general(xs_v[...], bre_v[...], NT, preferred_element_type=f32)
        if first:
            pin_wait(it, "bim", ur, PCOL["bim"])
        ui = lax.dot_general(xs_v[...], bim_v[...], NT, preferred_element_type=f32)
        if first:
            pin_wait(it, "wg", ui, PCOL["wg"])
        g = lax.dot_general(xs_v[...], wg_v[...], NT, preferred_element_type=f32)
        ln_early()
        if first:
            pin_wait(it, "wu", g, PCOL["wu"])
        else:
            acp(it).wait()
        u = lax.dot_general(xs_v[...], wu_v[...], NT, preferred_element_type=f32)
        a = (_gelu(g) * u).astype(bf16)
        if first:
            pin_wait(it, "wd", u, PCOL["wd"])
            pin_wait(it, "x", a, PCOL["x"])
        ln_late()
        z = None
        if SDEL[j] is not None:
            z = _zero_of(g[T - 8:, SDEL[j] * 128:(SDEL[j] + 1) * 128])
        hrb, hib, carry = scan(j, ur, ui, carry, z)
        res = xload(base2, j) + xs_v[...].astype(f32) * tab_v[5][0:1, :]
        y = res + jnp.dot(a, wd_v[...], preferred_element_type=f32)
        y = y + lax.dot_general(hrb, cre_v[...], NT, preferred_element_type=f32)
        y = y + lax.dot_general(hib, cim_v[...], NT, preferred_element_type=f32)
        r = pl.multiple_of(it * TI + OFF[j], 16)
        for c in range(NC):
            ot = o_v.at[c, pl.ds(r, T)]
            for k in range(Ls):
                ot[pl.ds(k, 8, stride=Ls), :] = y[8 * k:8 * k + 8, c * 128:(c + 1) * 128]
            ocp(it, j, c).start()
        return carry

    xa_v[pl.ds(0, TS[0])] = ln(0, 0)
    wait("bre")

    def body(it, carry):
        base2 = it * (TI // 2)

        def ln_b():
            xb_v[pl.ds(0, TS[1])] = ln(base2 + OFF[1] // 2, 1, NSER[0])

        def ln_next():
            nb = jnp.minimum(it + 1, NIT - 1) * (TI // 2)
            xa_v[pl.ds(0, TS[0])] = ln(nb, 0, NSER[1])

        carry = tile(it, 0, carry, True, lambda: None, ln_b)
        return tile(it, 1, carry, False, ln_next, lambda: None)

    lax.fori_loop(0, NIT, body, (jnp.zeros((8, P), f32), jnp.zeros((8, P), f32)))
    for it in range(NIT):
        for j in range(2):
            for c in range(NC):
                ocp(it, j, c).wait()


@jax.jit
def pallas_parallel_sum__ssm_conv_s5__geglu_ffn__prompt_kernel(
    A_x, A_Lambda_re, A_Lambda_im, A_B_re, A_B_im, A_C_re, A_C_im, A_log_dt, A_Dskip,
    B_x, B_w_gate, B_w_up, B_w_down,
):
    Bsz, S, D = A_x.shape
    P = A_Lambda_re.shape[0]
    F = B_w_gate.shape[1]
    x2 = A_x.reshape(Bsz * S, D)
    vec = lambda a: a.reshape(-1, 128)
    hbm = pl.BlockSpec(memory_space=pltpu.HBM)
    NC = D // 128
    STG = F + PADR + NIT * PADR
    out = pl.pallas_call(
        kernel,
        in_specs=[hbm] * 12,
        out_specs=hbm,
        out_shape=jax.ShapeDtypeStruct((S, D), f32),
        scratch_shapes=[
            pltpu.VMEM((NC, S + PADR, 128), bf16), pltpu.VMEM((4, P // 128, 128), bf16),
            pltpu.VMEM((P, D), bf16), pltpu.VMEM((P + PADR, D), bf16),
            pltpu.VMEM((D, P), bf16), pltpu.VMEM((D, P), bf16),
            pltpu.VMEM((F + PADR, D), bf16), pltpu.VMEM((STG + TA, D), bf16), pltpu.VMEM((STG + TA, D), bf16),
            pltpu.VMEM((NC, S, 128), f32),
            pltpu.VMEM((6 + 8 * len(LS), 8, P), f32), pltpu.VMEM((TA, D), bf16),
            pltpu.SemaphoreType.DMA((48,)),
        ],
        compiler_params=pltpu.CompilerParams(vmem_limit_bytes=100 * 1024 * 1024, flags=FL),
    )(x2, vec(A_Lambda_re), vec(A_Lambda_im), A_B_re, A_B_im, A_C_re, A_C_im,
      vec(A_log_dt), vec(A_Dskip), B_w_gate.T, B_w_up.T, B_w_down)
    return out.reshape(Bsz, S, D)
```

```python
import jax
import jax.numpy as jnp
from jax import lax
import jax.experimental.pallas as pl
import jax.experimental.pallas.tpu as pltpu

LS = (70, 58)
NIT = 2
BS = 256
GS = 640
PCOL = dict(bre2=0, bim=2, wg=1, wg2=1, wu=9, wd=8, x=9)
NSER = (12, 16)
SDEL = (None, 6)
NT = (((1,), (1,)), ((), ()))
f32 = jnp.float32
bf16 = jnp.bfloat16
u32 = jnp.uint32
PADR = 16
TA = 8 * max(LS)
NSEM = 15


def _gelu(x):
    c = 0.7978845608028654
    return 0.5 * x * (1.0 + jnp.tanh(c * (x + 0.044715 * (x * x * x))))


def _cmul(ar, ai, br, bi):
    return ar * br - ai * bi, ar * bi + ai * br


def _row(v):
    return jnp.concatenate([v[j:j + 1, :] for j in range(v.shape[0])], axis=1)


def _zero_of(v):
    z = lax.shift_right_logical(lax.clz(pltpu.bitcast(v[0:8, 0:128], u32)), jnp.uint32(6))
    return z[0:1, 0:1]


def _after(v, z):
    return pltpu.bitcast(pltpu.bitcast(v, u32) | z, f32)


def kernel(x_hbm, lre_hbm, lim_hbm, bre_hbm, bim_hbm, cre_hbm, cim_hbm, ldt_hbm, dsk_hbm,
           wg_hbm, wu_hbm, wd_hbm, o_hbm,
           x_v, vec_v, bre_f, bim_f, cre_v, cim_v, wg_f, wu_f, wd_f, o_v, tab_v, sems):
    S, D = x_hbm.shape
    P = D
    F = wg_hbm.shape[0]
    NC = D // 128
    TS = [8 * l for l in LS]
    TI = sum(TS)
    assert TI * NIT == S
    OFF = [0, TS[0]]

    cnt = [0]

    def nsem():
        cnt[0] += 1
        return cnt[0] - 1

    def cp(src, dst, k):
        return pltpu.make_async_copy(src, dst, sems.at[k])

    bre_v, bim_v = bre_f.at[pl.ds(0, P)], bim_f.at[pl.ds(0, P)]
    wg_v, wu_v, wd_v = wg_f.at[pl.ds(0, F)], wu_f.at[pl.ds(0, F)], wd_f.at[pl.ds(0, F)]
    DUM = F + PADR
    STG = DUM + NIT * PADR
    xa_v = wu_f.at[pl.ds(STG, TA)]
    xb_v = wd_f.at[pl.ds(STG, TA)]

    x0_sem, x_sem, o_sem, vec_sem = nsem(), nsem(), nsem(), nsem()
    a_sem = [nsem() for _ in range(NIT)]

    def xcps(t):
        r, n = (t // 2) * TI + OFF[t % 2], TS[t % 2]
        return [cp(x_hbm.at[pl.ds(r, n), pl.ds(c * 128, 128)], x_v.at[c, pl.ds(r, n)], x0_sem if t == 0 else x_sem)
                for c in range(NC)]

    def ocp(it, j, c):
        r = it * TI + OFF[j]
        if not isinstance(it, int):
            r = pl.multiple_of(r, 16)
        return cp(o_v.at[c, pl.ds(r, TS[j])], o_hbm.at[pl.ds(r, TS[j]), pl.ds(c * 128, 128)], o_sem)

    def acp(it):
        r = DUM + it * PADR
        if isinstance(it, int):
            return cp(wu_hbm.at[pl.ds(0, PADR)], wu_f.at[pl.ds(r, PADR)], a_sem[it])
        r = pl.multiple_of(r, PADR)
        return cp(wu_hbm.at[pl.ds(0, PADR)], wu_f.at[pl.ds(r, PADR)], a_sem[0] + it)

    G = dict(
        vec=[cp(lre_hbm, vec_v.at[0], vec_sem), cp(lim_hbm, vec_v.at[1], vec_sem),
             cp(ldt_hbm, vec_v.at[2], vec_sem), cp(dsk_hbm, vec_v.at[3], vec_sem)],
        x0=xcps(0),
        bre=[cp(bre_hbm.at[pl.ds(0, BS)], bre_v.at[pl.ds(0, BS)], nsem())],
        bre2=[cp(bre_hbm.at[pl.ds(BS, P - BS)], bre_v.at[pl.ds(BS, P - BS)], nsem())],
        bim=[cp(bim_hbm, bim_v, nsem())],
        wg=[cp(wg_hbm.at[pl.ds(0, GS)], wg_v.at[pl.ds(0, GS)], nsem())],
        wg2=[cp(wg_hbm.at[pl.ds(GS, F - GS)], wg_v.at[pl.ds(GS, F - GS)], nsem())],
        wu=[cp(wu_hbm, wu_v, nsem())],
        wd=[cp(wd_hbm, wd_v, nsem()), cp(cre_hbm, cre_v, nsem()), cp(cim_hbm, cim_v, nsem())],
        x=[c for t in range(1, 2 * NIT) for c in xcps(t)],
    )
    assert cnt[0] == NSEM
    for n in ("vec", "x0", "bre", "bre2", "bim", "wg", "wg2", "wu", "wd", "x"):
        for c in G[n]:
            c.start()
    for it in range(NIT):
        acp(it).start()

    def wait(n):
        for c in G[n]:
            c.wait()

    def pin_wait(it, n, val, j):
        v = val[val.shape[0] - 16:, j * 128:(j + 1) * 128].astype(bf16)
        spare = dict(bre2=bre_f.at[pl.ds(P + PADR, PADR), pl.ds(0, 128)],
                     bim=bim_f.at[pl.ds(P, PADR), pl.ds(0, 128)],
                     wg=wg_f.at[pl.ds(F, PADR), pl.ds(0, 128)],
                     wg2=wg_f.at[pl.ds(F + PADR, PADR), pl.ds(0, 128)],
                     wu=wu_f.at[pl.ds(F, PADR), pl.ds(0, 128)],
                     wd=wd_f.at[pl.ds(F, PADR), pl.ds(0, 128)],
                     x=x_v.at[1, pl.ds(S, PADR)])[n]
        spare[...] = v

        @pl.when(it == 0)
        def _():
            wait(n)

    wait("vec")

    lre = vec_v[0].astype(f32)
    lim = vec_v[1].astype(f32)
    dt = jnp.exp(vec_v[2].astype(f32)).astype(vec_v.dtype).astype(f32)
    wr = dt * lre
    wi = dt * lim
    mag = jnp.exp(wr)
    a_r = mag * jnp.cos(wi)
    a_i = mag * jnp.sin(wi)
    den = lre * lre + lim * lim
    nr = a_r - 1.0
    cf_r = 2.0 * ((nr * lre + a_i * lim) / den)
    cf_i = 2.0 * ((a_i * lre - nr * lim) / den)
    bc = lambda v: jnp.broadcast_to(_row(v), (8, P))
    row = lax.broadcasted_iota(jnp.int32, (8, P), 0)
    tab_v[0], tab_v[1] = bc(a_r), bc(a_i)
    tab_v[2], tab_v[3], tab_v[4] = bc(cf_r), bc(cf_i), bc(-cf_r)
    tab_v[5] = bc(vec_v[3].astype(f32))
    for j, Ls in enumerate(LS):
        magL = jnp.exp(Ls * wr)
        Ar, Ai = bc(magL * jnp.cos(Ls * wi)), bc(magL * jnp.sin(Ls * wi))
        A2 = _cmul(Ar, Ai, Ar, Ai)
        A4 = _cmul(*A2, *A2)
        b = 6 + 8 * j
        tab_v[b], tab_v[b + 1] = Ar, Ai
        for q, (s, (mr, mi)) in enumerate(((1, (Ar, Ai)), (2, A2), (4, A4))):
            tab_v[b + 2 + 2 * q] = jnp.where(row >= s, mr, 0.0)
            tab_v[b + 3 + 2 * q] = jnp.where(row >= s, mi, 0.0)

    x_v[0, pl.ds(S, PADR), :] = jnp.concatenate([A4[0][:, 0:128], A4[1][:, 0:128]], axis=0).astype(bf16)
    wait("x0")
    xw = [x_v.at[c].bitcast(u32) for c in range(NC)]

    def xload(base2, j):
        Ls = LS[j]
        if not isinstance(base2, int):
            base2 = pl.multiple_of(base2, 8)
        xt = [xw[c].at[pl.ds(base2, 4 * Ls)] for c in range(NC)]
        parts = []
        for k in range(Ls // 2):
            w = jnp.concatenate([xt[c][pl.ds(k, 8, stride=Ls // 2), :] for c in range(NC)], axis=1)
            parts.append(pltpu.bitcast(w << 16, f32))
            parts.append(pltpu.bitcast(w & jnp.uint32(0xFFFF0000), f32))
        return jnp.concatenate(parts, axis=0)

    def ln(base2, j, nser=1):
        x = xload(base2, j)
        nb = x.shape[0] // 16
        edges = [16 * ((nb * q) // nser) for q in range(nser + 1)]
        outs, z = [], None
        for q in range(nser):
            xq = x[edges[q]:edges[q + 1]]
            m = jnp.mean(xq, axis=-1, keepdims=True)
            if z is not None:
                m = _after(m, z)
            xc = xq - m
            v = jnp.mean(xc * xc, axis=-1, keepdims=True)
            xn = xc * lax.rsqrt(v + 1e-5)
            z = _zero_of(xn)
            outs.append(xn.astype(bf16))
        return jnp.concatenate(outs, axis=0) if nser > 1 else outs[0]

    def scan(j, ur, ui, carry, z=None):
        Ls = LS[j]
        b = 6 + 8 * j
        us = [(ur[8 * k:8 * k + 8], ui[8 * k:8 * k + 8]) for k in range(Ls)]
        ar, ai = tab_v[0], tab_v[1]
        er, ei = us[0]
        if z is not None:
            er, ei = _after(er, z), _after(ei, z)
        for k in range(1, Ls):
            tr, ti = _cmul(ar, ai, er, ei)
            er, ei = tr + us[k][0], ti + us[k][1]
        zr = jnp.where(row == 0, carry[0], pltpu.roll(er, 1, 0))
        zi = jnp.where(row == 0, carry[1], pltpu.roll(ei, 1, 0))
        for t, sh in enumerate((1, 2, 4)):
            tr, ti = _cmul(tab_v[b + 2 + 2 * t], tab_v[b + 3 + 2 * t], pltpu.roll(zr, sh, 0), pltpu.roll(zi, sh, 0))
            zr, zi = zr + tr, zi + ti
        tr, ti = _cmul(tab_v[b], tab_v[b + 1], zr, zi)
        carry = (pltpu.roll(tr + er, 1, 0), pltpu.roll(ti + ei, 1, 0))
        hr, hi = zr, zi
        hrs, his = [], []
        cr, ci, ncr = tab_v[2], tab_v[3], tab_v[4]
        for k in range(Ls):
            tr, ti = _cmul(ar, ai, hr, hi)
            hr, hi = tr + us[k][0], ti + us[k][1]
            hrs.append(cr * hr - ci * hi)
            his.append(ncr * hi - ci * hr)
        return jnp.concatenate(hrs, axis=0).astype(bf16), jnp.concatenate(his, axis=0).astype(bf16), carry

    def tile(it, j, carry, first, ln_early, ln_late):
        T = TS[j]
        Ls = LS[j]
        base2 = it * (TI // 2) + OFF[j] // 2
        xs_v = (xa_v, xb_v)[j].at[pl.ds(0, T)]
        dot = lambda w: lax.dot_general(xs_v[...], w, NT, preferred_element_type=f32)
        if first:
            ur0 = dot(bre_v[0:BS])
            pin_wait(it, "bre2", ur0, PCOL["bre2"])
            ur = jnp.concatenate([ur0, dot(bre_v[BS:P])], axis=1)
            pin_wait(it, "bim", ur, PCOL["bim"])
            ui = dot(bim_v[...])
            pin_wait(it, "wg", ui, PCOL["wg"])
            g0 = dot(wg_v[0:GS])
            pin_wait(it, "wg2", g0, PCOL["wg2"])
            g = jnp.concatenate([g0, dot(wg_v[GS:F])], axis=1)
            pin_wait(it, "wu", g, PCOL["wu"])
        else:
            ur = dot(bre_v[...])
            ui = dot(bim_v[...])
            g = dot(wg_v[...])
            ln_early()
            acp(it).wait()
        u = dot(wu_v[...])
        a = (_gelu(g) * u).astype(bf16)
        if first:
            pin_wait(it, "wd", u, PCOL["wd"])
            pin_wait(it, "x", a, PCOL["x"])
        ln_late()
        z = None
        if SDEL[j] is not None:
            z = _zero_of(g[T - 8:, SDEL[j] * 128:(SDEL[j] + 1) * 128])
        hrb, hib, carry = scan(j, ur, ui, carry, z)
        res = xload(base2, j) + xs_v[...].astype(f32) * tab_v[5][0:1, :]
        y = res + jnp.dot(a, wd_v[...], preferred_element_type=f32)
        y = y + lax.dot_general(hrb, cre_v[...], NT, preferred_element_type=f32)
        y = y + lax.dot_general(hib, cim_v[...], NT, preferred_element_type=f32)
        r = pl.multiple_of(it * TI + OFF[j], 16)
        for c in range(NC):
            ot = o_v.at[c, pl.ds(r, T)]
            for k in range(Ls):
                ot[pl.ds(k, 8, stride=Ls), :] = y[8 * k:8 * k + 8, c * 128:(c + 1) * 128]
            ocp(it, j, c).start()
        return carry

    xn0 = ln(0, 0)
    xa_v[pl.ds(0, TS[0])] = xn0
    w0 = pltpu.bitcast(xn0, u32)[:, 0:128]
    acc = w0[0:8]
    for r in range(8, w0.shape[0], 8):
        acc = acc | w0[r:r + 8]
    bre_f[pl.ds(P, PADR), 0:128] = pltpu.bitcast(acc, bf16)
    wait("bre")

    def body(it, carry):
        base2 = it * (TI // 2)

        def ln_b():
            xb_v[pl.ds(0, TS[1])] = ln(base2 + OFF[1] // 2, 1, NSER[0])

        def ln_next():
            nb = jnp.minimum(it + 1, NIT - 1) * (TI // 2)
            xa_v[pl.ds(0, TS[0])] = ln(nb, 0, NSER[1])

        carry = tile(it, 0, carry, True, None, ln_b)
        return tile(it, 1, carry, False, ln_next, lambda: None)

    lax.fori_loop(0, NIT, body, (jnp.zeros((8, P), f32), jnp.zeros((8, P), f32)))
    for it in range(NIT):
        for j in range(2):
            for c in range(NC):
                ocp(it, j, c).wait()


@jax.jit
def pallas_parallel_sum__ssm_conv_s5__geglu_ffn__prompt_kernel(
    A_x: jax.Array,
    A_Lambda_re: jax.Array,
    A_Lambda_im: jax.Array,
    A_B_re: jax.Array,
    A_B_im: jax.Array,
    A_C_re: jax.Array,
    A_C_im: jax.Array,
    A_log_dt: jax.Array,
    A_Dskip: jax.Array,
    B_x: jax.Array,
    B_w_gate: jax.Array,
    B_w_up: jax.Array,
    B_w_down: jax.Array,
):
    Bsz, S, D = A_x.shape
    P = A_Lambda_re.shape[0]
    F = B_w_gate.shape[1]
    assert Bsz == 1 and P == D
    x2 = A_x.reshape(Bsz * S, D)
    vec = lambda a: a.reshape(-1, 128)
    hbm = pl.BlockSpec(memory_space=pltpu.HBM)
    NC = D // 128
    STG = F + PADR + NIT * PADR
    dt = A_x.dtype
    out = pl.pallas_call(
        kernel,
        in_specs=[hbm] * 12,
        out_specs=hbm,
        out_shape=jax.ShapeDtypeStruct((S, D), f32),
        scratch_shapes=[
            pltpu.VMEM((NC, S + PADR, 128), dt), pltpu.VMEM((4, P // 128, 128), dt),
            pltpu.VMEM((P + 2 * PADR, D), dt), pltpu.VMEM((P + PADR, D), dt),
            pltpu.VMEM((D, P), dt), pltpu.VMEM((D, P), dt),
            pltpu.VMEM((F + 2 * PADR, D), dt), pltpu.VMEM((STG + TA, D), dt), pltpu.VMEM((STG + TA, D), dt),
            pltpu.VMEM((NC, S, 128), f32),
            pltpu.VMEM((6 + 8 * len(LS), 8, P), f32),
            pltpu.SemaphoreType.DMA((NSEM,)),
        ],
        compiler_params=pltpu.CompilerParams(
            vmem_limit_bytes=64 * 1024 * 1024,
            flags={"XLA_TPU_RESCHEDULE_DMA_DONES": True},
            disable_semaphore_checks=True),
    )(x2, vec(A_Lambda_re), vec(A_Lambda_im), A_B_re, A_B_im, A_C_re, A_C_im,
      vec(A_log_dt), vec(A_Dskip), B_w_gate.T, B_w_up.T, B_w_down)
    return out.reshape(Bsz, S, D)
```
